```python
import os as _os
_os.environ.setdefault("JAX_PLATFORMS", "cpu")
import jax
import jax.numpy as jnp

def _softmax(x, axis=-1):
    return jax.nn.softmax(x, axis=axis)
def _gelu(x):
    return jax.nn.gelu(x, approximate=True)
def _silu(x):
    return jax.nn.silu(x)
def _sigmoid(x):
    return jax.nn.sigmoid(x)
def _layernorm(x, axis=-1, eps=1e-5):
    m = jnp.mean(x, axis=axis, keepdims=True)
    v = jnp.var(x, axis=axis, keepdims=True)
    return (x - m) / jnp.sqrt(v + eps)
def _scatter_add(tgt, idx, src, axis=0):
    return tgt.at[idx].add(src)
def _segment_sum(src, seg, n):
    return jax.ops.segment_sum(src, seg, n)
class _Rng:
    def __init__(self, key):
        self._k = key
    def _next(self):
        self._k, sub = jax.random.split(self._k)
        return sub
    def normal(self, shape):
        return jax.random.normal(self._next(), shape, dtype=jnp.bfloat16)
    def randint(self, lo, hi, shape):
        return jax.random.randint(self._next(), shape, lo, hi, dtype=jnp.int32)
    def uniform(self, shape, lo=0.0, hi=1.0):
        return jax.random.uniform(self._next(), shape, jnp.bfloat16, lo, hi)
    def permutation(self, n):
        return jax.random.permutation(self._next(), n)


kernel_name = 'standalone__sliding_block_cached__sampling'

def setup_inputs():
    _rng = _Rng(jax.random.key(int.from_bytes(__import__("os").urandom(4), "little")))
    _w = (lambda a: (lambda t: t.astype(jnp.bfloat16) if jnp.issubdtype(t.dtype, jnp.floating) else t)(jnp.asarray(a)))
    B, Sq, D = 8, 4, 640
    Hq, Hkv, Sk, Dh = 32, 32, 4096, 192
    assert Hq % Hkv == 0, (Hq, Hkv)
    return {
        "x": _w((lambda *s: _rng.normal(s) * 0.8)(B, Sq, D)),
        "k_cache": _w((lambda *s: _rng.normal(s) * 0.8)(B, Hkv, Sk, Dh)),
        "v_cache": _w((lambda *s: _rng.normal(s) * 0.05)(B, Hkv, Sk, Dh)),
        "wq": _w((lambda *s: _rng.normal(s) * 0.8)(D, Hq * Dh) * (D ** -0.5)),
        "wo": _w((lambda *s: _rng.normal(s) * 0.05)(Hq * Dh, D) * ((Hq * Dh) ** -0.5)),
    }

def reference(x, k_cache, v_cache, wq, wo):
    B, Sq, D = x.shape
    Hq, Dh = 32, 192
    Hkv, Sk = k_cache.shape[1], k_cache.shape[2]
    W = min(4096, max(256, Sk // 4))
    rep = Hq // Hkv
    q = (lambda x, *d: x.transpose(*d))((x @ wq).reshape(B, Sq, Hq, Dh), 0, 2, 1, 3)
    k = jnp.repeat(k_cache[:, :, Sk - W:, :], rep, axis=1)
    v = jnp.repeat(v_cache[:, :, Sk - W:, :], rep, axis=1)
    scores = jnp.einsum("bhqd,bhkd->bhqk", q, k) * (Dh ** -0.5)
    p = _softmax(scores, axis=-1)
    o = jnp.einsum("bhqk,bhkd->bhqd", p, v)
    return (lambda x, *d: x.transpose(*d))(o, 0, 2, 1, 3).reshape(B, Sq, Hq * Dh) @ wo
```

```python
import jax
import jax.numpy as jnp
import jax.experimental.pallas as pl
import jax.experimental.pallas.tpu as pltpu

_HQ, _DH = 32, 192
_PAIR = 2 * _DH
_SUB = 16
_STREAMS = 4
_LOOKAHEAD = 4
_SLOTS = _LOOKAHEAD + 1


def _aligned(v, m):
    return v if isinstance(v, int) else pl.multiple_of(v, m)


@jax.jit
def pallas_standalone__sliding_block_cached__sampling_kernel(
    x: jax.Array,
    k_cache: jax.Array,
    v_cache: jax.Array,
    wq: jax.Array,
    wo: jax.Array,
):
    B, Sq, D = x.shape
    Hkv, Sk = k_cache.shape[1], k_cache.shape[2]
    assert Hkv == _HQ and k_cache.shape[3] == _DH and Sq == 4
    W = min(4096, max(256, Sk // 4))
    G = _HQ // 2
    N = G * B
    M = 2 * Sq
    scale = _DH ** -0.5
    wq_rows, wo_rows = D // (2 * B), _PAIR // (2 * B)
    per = _PAIR // _SUB // _STREAMS
    order = [t * per + j for j in range(per) for t in range(_STREAMS)]

    def kernel_function(x_hbm, k_hbm, v_hbm, wq_hbm, wo_hbm, o_ref,
                        x_buf, k_buf, v_buf, wq_buf, wo_buf, x2, q_scr, o_scr, acc,
                        x_sem, k_sem, v_sem, wq_sem, wo_sem):
        def start_wq(g, b):
            for j in range(2):
                r0 = _aligned((2 * b + j) * wq_rows, 8)
                pltpu.make_async_copy(
                    wq_hbm.at[pl.ds(r0, wq_rows), pl.ds(_aligned(g * _PAIR, 128), _PAIR)],
                    wq_buf.at[g % 2, pl.ds(r0, wq_rows), :],
                    wq_sem.at[g % 2]).start(priority=j)

        def start_wo(g, b):
            for j in range(2):
                r0 = _aligned((2 * b + j) * wo_rows, 8)
                pltpu.make_async_copy(
                    wo_hbm.at[pl.ds(_aligned(g * _PAIR + r0, 8), wo_rows), :],
                    wo_buf.at[g % 2, pl.ds(r0, wo_rows), :],
                    wo_sem.at[g % 2]).start(priority=j)

        def start_chunk(i):
            g, b, slot = i // B, i % B, i % _SLOTS
            start_wo(g, b)
            if isinstance(g, int):
                if g + 1 < G:
                    start_wq(g + 1, b)
            else:
                pl.when(g + 1 < G)(lambda: start_wq(g + 1, b))
            for s in order:
                r0 = _aligned(g * _PAIR + s * _SUB, 8)
                for prio, (src, buf, sem) in enumerate(
                        ((k_hbm, k_buf, k_sem), (v_hbm, v_buf, v_sem))):
                    pltpu.make_async_copy(
                        src.at[b, pl.ds(r0, _SUB), pl.ds(Sk - W, W)],
                        buf.at[slot, pl.ds(s * _SUB, _SUB), :],
                        sem.at[slot]).start(priority=prio)

        def wait_slot(buf, sem, slot):
            pltpu.make_async_copy(buf.at[slot], buf.at[slot], sem.at[slot]).wait()

        x_copy = pltpu.make_async_copy(x_hbm, x_buf, x_sem)
        x_copy.start()
        for b in range(B):
            start_wq(0, b)
        for i in range(_LOOKAHEAD):
            start_chunk(i)
        x_copy.wait()
        for b in range(B):
            xb = x_buf[b].astype(jnp.float32)
            x2[b * M:b * M + Sq, :] = xb
            x2[b * M + Sq:(b + 1) * M, :] = xb
        acc[...] = jnp.zeros_like(acc)

        def own_head(rows):
            r = jax.lax.broadcasted_iota(jnp.int32, (rows, _PAIR), 0)
            c = jax.lax.broadcasted_iota(jnp.int32, (rows, _PAIR), 1)
            return ((r % M) < Sq) == (c < _DH)

        def pair_body(g, carry):
            ws = g % 2
            wait_slot(wq_buf, wq_sem, ws)
            q = jnp.dot(x2[...].astype(jnp.bfloat16), wq_buf[ws],
                        preferred_element_type=jnp.float32)
            q_scr[...] = jnp.where(own_head(B * M), q, 0.0)

            def batch_body(b, carry):
                i = g * B + b
                pl.when(i + _LOOKAHEAD < N)(lambda: start_chunk(i + _LOOKAHEAD))
                slot = i % _SLOTS
                rows = pl.ds(pl.multiple_of(b * M, M), M)
                wait_slot(k_buf, k_sem, slot)
                s = jnp.dot(q_scr[rows, :].astype(jnp.bfloat16), k_buf[slot],
                            preferred_element_type=jnp.float32) * scale
                e = jnp.exp(s - jnp.max(s, axis=-1, keepdims=True))
                denom = jnp.sum(e, axis=-1, keepdims=True)
                wait_slot(v_buf, v_sem, slot)
                o = jax.lax.dot_general(e.astype(jnp.bfloat16), v_buf[slot],
                                        (((1,), (1,)), ((), ())),
                                        preferred_element_type=jnp.float32)
                o_scr[rows, :] = jnp.where(own_head(M), o / denom, 0.0)
                return carry

            jax.lax.fori_loop(0, B, batch_body, 0)
            wait_slot(wo_buf, wo_sem, ws)
            acc[...] += jnp.dot(o_scr[...].astype(jnp.bfloat16), wo_buf[ws],
                                preferred_element_type=jnp.float32)
            return carry

        jax.lax.fori_loop(0, G, pair_body, 0)
        for b in range(B):
            o_ref[b] = (acc[b * M:b * M + Sq, :]
                        + acc[b * M + Sq:(b + 1) * M, :]).astype(o_ref.dtype)

    k_t = jnp.swapaxes(k_cache, 2, 3).reshape(B, Hkv * _DH, Sk)
    v_t = jnp.swapaxes(v_cache, 2, 3).reshape(B, Hkv * _DH, Sk)
    return pl.pallas_call(
        kernel_function,
        in_specs=[pl.BlockSpec(memory_space=pl.ANY)] * 5,
        out_specs=pl.BlockSpec(memory_space=pltpu.VMEM),
        out_shape=jax.ShapeDtypeStruct((B, Sq, D), x.dtype),
        scratch_shapes=[
            pltpu.VMEM((B, Sq, D), x.dtype),
            pltpu.VMEM((_SLOTS, _PAIR, W), k_cache.dtype),
            pltpu.VMEM((_SLOTS, _PAIR, W), v_cache.dtype),
            pltpu.VMEM((2, D, _PAIR), wq.dtype),
            pltpu.VMEM((2, _PAIR, D), wo.dtype),
            pltpu.VMEM((B * M, D), jnp.float32),
            pltpu.VMEM((B * M, _PAIR), jnp.float32),
            pltpu.VMEM((B * M, _PAIR), jnp.float32),
            pltpu.VMEM((B * M, D), jnp.float32),
            pltpu.SemaphoreType.DMA(()),
            pltpu.SemaphoreType.DMA((_SLOTS,)),
            pltpu.SemaphoreType.DMA((_SLOTS,)),
            pltpu.SemaphoreType.DMA((2,)),
            pltpu.SemaphoreType.DMA((2,)),
        ],
        compiler_params=pltpu.CompilerParams(vmem_limit_bytes=64 * 2**20),
    )(x, k_t, v_t, wq, wo)
```

```python
import jax
import jax.numpy as jnp
import jax.experimental.pallas as pl
import jax.experimental.pallas.tpu as pltpu

_HQ, _DH = 32, 192
_PAIR = 2 * _DH
_TILE = 128
_TPP = _PAIR // _TILE
_ROWS = 8
_RING = 128
_SEMS = 8
_AHEAD = 5
_EXTRA = 3
_WQ_COLS, _WQ_STREAMS = 1536, 8
_WO_ROWS = 16
_WO_EARLY = 4
_WO_LAST = (2, 1, 2, 1, 2, 1)


def _aligned(v, m):
    return v if isinstance(v, int) else pl.multiple_of(v, m)


@jax.jit
def pallas_standalone__sliding_block_cached__sampling_kernel(
    x: jax.Array,
    k_cache: jax.Array,
    v_cache: jax.Array,
    wq: jax.Array,
    wo: jax.Array,
):
    B, Sq, D = x.shape
    Hkv, Sk = k_cache.shape[1], k_cache.shape[2]
    assert (B, Sq, Hkv, k_cache.shape[3]) == (8, 4, _HQ, _DH) and D % _TILE == 0
    W = min(4096, max(256, Sk // 4))
    scale = _DH ** -0.5
    M = 2 * Sq
    G = _HQ // 2
    SPG = _PAIR // _ROWS
    STAGES = SPG // B
    NKV = G * SPG
    assert STAGES == 2 * _TPP == len(_WO_LAST)
    assert 2 * SPG + _AHEAD + 1 <= _RING and _AHEAD + 2 <= _SEMS - 1
    wq_blocks = _HQ * _DH // _WQ_COLS
    wq_per_stream = (D // 8) * wq_blocks // _WQ_STREAMS
    UPS = _TILE // _WO_ROWS
    NU = G * UPS
    wo_last = [sum(_WO_LAST[:t]) for t in range(STAGES + 1)]
    wo_rest = _AHEAD * _WO_EARLY + B * wo_last[STAGES]
    wo_per_step = pl.cdiv(NU - wo_rest, _SEMS)
    assert UPS == 8 and G == 2 * _SEMS and _SEMS * UPS <= wo_rest <= NU
    for b in range(B):
        assert (_AHEAD * _WO_EARLY + (b + 1) * wo_last[STAGES] - 1) // UPS < _SEMS + max(0, b - 3)

    def kernel_function(x_hbm, k_hbm, v_hbm, wq_hbm, wo_hbm, o_ref,
                        x_buf, kv_buf, wq_buf, wo_buf, x2, q_scr, o_scr, sems):
        def wait_all(dst, sem):
            pltpu.make_async_copy(dst, dst, sem).wait()

        def start_wq(j, carry):
            for s in range(_WQ_STREAMS):
                n = s * wq_per_stream + j
                piece = (pl.ds(_aligned((n // wq_blocks) * 8, 8), 8),
                         pl.ds(_aligned((n % wq_blocks) * _WQ_COLS, _TILE), _WQ_COLS))
                pltpu.make_async_copy(wq_hbm.at[piece], wq_buf.at[piece],
                                      sems.at[_SEMS - 2]).start(priority=s % 2)
            return carry

        def ring_rows(u):
            return pl.ds(_aligned((u & (_RING - 1)) * _ROWS, _ROWS), _ROWS)

        def start_kv(u, batches):
            for b in batches:
                for t, src in ((1, v_hbm), (0, k_hbm)):
                    pltpu.make_async_copy(
                        src.at[b, pl.ds(_aligned(u * _ROWS, _ROWS), _ROWS), pl.ds(Sk - W, W)],
                        kv_buf.at[t, b, ring_rows(u), :],
                        sems.at[u & (_SEMS - 1)]).start(priority=1 - t)

        def wait_kv(u):
            wait_all(kv_buf.at[:, :, ring_rows(u), :], sems.at[u & (_SEMS - 1)])

        def kv_step(u):
            start_kv(u + _AHEAD, range(_EXTRA, B))
            wait_kv(u)
            start_kv(u + _AHEAD + 1, range(_EXTRA))

        def start_wo(m, parity):
            j, rows = m >> 3, pl.ds(_aligned((m & (UPS - 1)) * _WO_ROWS, _WO_ROWS), _WO_ROWS)
            for s in range(_TPP):
                pltpu.make_async_copy(wo_hbm.at[s, j, rows, :], wo_buf.at[s, j, rows, :],
                                      sems.at[j & (_SEMS - 1)]).start(priority=(parity + s) % 2)

        def wait_wo(j):
            wait_all(wo_buf.at[:, j], sems.at[j & (_SEMS - 1)])

        def own_head(rows, t):
            r = jax.lax.broadcasted_iota(jnp.int32, (rows, _TILE), 0)
            c = jax.lax.broadcasted_iota(jnp.int32, (rows, _TILE), 1) + t * _TILE
            return ((r & (M - 1)) < Sq) == (c < _DH)

        def attend(g, b, before_stage):
            q_rows = pl.ds(_aligned(b * M, M), M)
            o_rows = pl.ds(_aligned((b >> 1) * M, M), M)

            def tile(t):
                return pl.ds(_aligned(((g * _TPP + t) & (_RING * _ROWS // _TILE - 1)) * _TILE, _TILE),
                             _TILE)

            s = None
            for t in range(_TPP):
                before_stage(t)
                part = jnp.dot(q_scr[g * _TPP + t, q_rows, :].astype(kv_buf.dtype),
                               kv_buf[0, b, tile(t), :], preferred_element_type=jnp.float32)
                s = part if s is None else s + part
            s = s * scale
            e = jnp.exp(s - jnp.max(s, axis=-1, keepdims=True))
            denom = jnp.sum(e, axis=-1, keepdims=True)
            e = e.astype(kv_buf.dtype)
            half = (jax.lax.broadcasted_iota(jnp.int32, (M, _TILE), 0) >> 2) == (b & 1)
            for t in range(_TPP):
                before_stage(_TPP + t)
                o = jax.lax.dot_general(e, kv_buf[1, b, tile(t), :], (((1,), (1,)), ((), ())),
                                        preferred_element_type=jnp.float32) / denom
                o = jnp.where(own_head(M, t), o, pltpu.roll(o, Sq, 0))
                pltpu.store(o_scr.at[g * _TPP + t, o_rows, :], o, mask=half)

        pltpu.make_async_copy(x_hbm, x_buf, sems.at[_SEMS - 1]).start()
        jax.lax.fori_loop(0, wq_per_stream, start_wq, 0)

        def first_steps(u, carry):
            start_kv(u, range(B))
            return carry

        jax.lax.fori_loop(0, _AHEAD, first_steps, 0)
        start_kv(_AHEAD, range(_EXTRA))
        wait_all(x_buf, sems.at[_SEMS - 1])
        for b in range(B):
            xb = x_buf[b].astype(jnp.float32)
            x2[b * M:(b + 1) * M, :] = jnp.concatenate([xb, xb], axis=0).astype(x2.dtype)
        wait_all(wq_buf, sems.at[_SEMS - 2])

        def project_q(g, carry):
            for t in range(_TPP):
                kv_step(g * _TPP + t)
                cols = pl.ds(_aligned(g * _PAIR + t * _TILE, _TILE), _TILE)
                q = jnp.dot(x2[...], wq_buf[:, cols], preferred_element_type=jnp.float32)
                q_scr[g * _TPP + t] = jnp.where(own_head(B * M, t), q, 0.0)
            return carry

        jax.lax.fori_loop(0, G, project_q, 0)

        def chunk(i, carry):
            attend(i >> 3, i & (B - 1), lambda t: kv_step(SPG + STAGES * i + t))
            return carry

        last = (G - 1) * B - 1
        jax.lax.fori_loop(0, last, chunk, 0)

        def final_kv_step(t):
            u = SPG + STAGES * last + t
            if u + _AHEAD < NKV:
                start_kv(u + _AHEAD, range(_EXTRA, B))
            else:
                for n in range(_WO_EARLY):
                    start_wo((u + _AHEAD - NKV) * _WO_EARLY + n, n)
            wait_kv(u)

        assert _AHEAD + 1 == STAGES
        attend(last // B, last % B, final_kv_step)

        def last_pair(b, carry):
            pl.when(b >= 4)(lambda: wait_wo(b - 4))

            def wo_stage(t):
                for n in range(wo_last[t], wo_last[t + 1]):
                    start_wo(_AHEAD * _WO_EARLY + b * wo_last[STAGES] + n, n)

            attend(G - 1, b, wo_stage)
            return carry

        jax.lax.fori_loop(0, B, last_pair, 0)
        for j in range(B - 4, _SEMS):
            wait_wo(j)

        def project_out(j, acc):
            @pl.when(j < _SEMS)
            def _():
                for n in range(wo_per_step):
                    m = wo_rest + j * wo_per_step + n
                    if wo_rest + (_SEMS - 1) * wo_per_step + n < NU:
                        start_wo(m, n)
                    else:
                        pl.when(m < NU)(lambda m=m, n=n: start_wo(m, n))

            pl.when(j >= _SEMS)(lambda: wait_wo(j))
            out = None
            for s in range(_TPP):
                part = jnp.dot(o_scr[s * G + j].astype(wo_buf.dtype), wo_buf[s, j],
                               preferred_element_type=jnp.float32)
                out = part if out is None else out + part
            return acc + out

        acc = jax.lax.fori_loop(0, G, project_out, jnp.zeros((B * Sq, D), jnp.float32))
        for b in range(B):
            o_ref[b] = acc[b * Sq:(b + 1) * Sq, :].astype(o_ref.dtype)

    k_t = jnp.swapaxes(k_cache, 2, 3).reshape(B, Hkv * _DH, Sk)
    v_t = jnp.swapaxes(v_cache, 2, 3).reshape(B, Hkv * _DH, Sk)
    return pl.pallas_call(
        kernel_function,
        in_specs=[pl.BlockSpec(memory_space=pl.ANY)] * 5,
        out_specs=pl.BlockSpec(memory_space=pltpu.VMEM),
        out_shape=jax.ShapeDtypeStruct((B, Sq, D), x.dtype),
        scratch_shapes=[
            pltpu.VMEM((B, Sq, D), x.dtype),
            pltpu.VMEM((2, B, _RING * _ROWS, W), k_cache.dtype),
            pltpu.VMEM(wq.shape, wq.dtype),
            pltpu.VMEM((_TPP, G, _TILE, D), wo.dtype),
            pltpu.VMEM((B * M, D), x.dtype),
            pltpu.VMEM((G * _TPP, B * M, _TILE), jnp.float32),
            pltpu.VMEM((G * _TPP, B * Sq, _TILE), jnp.float32),
            pltpu.SemaphoreType.DMA((_SEMS,)),
        ],
        compiler_params=pltpu.CompilerParams(vmem_limit_bytes=64 * 2**20),
    )(x, k_t, v_t, wq, wo.reshape(_TPP, G, _TILE, D))
```
